```python
import os as _os
_os.environ.setdefault('JAX_PLATFORMS', 'cpu')
import jax
import jax.numpy as jnp

def _softmax(x, axis=-1):
    return jax.nn.softmax(x, axis=axis)

def _gelu(x):
    return jax.nn.gelu(x, approximate=True)

def _silu(x):
    return jax.nn.silu(x)

def _sigmoid(x):
    return jax.nn.sigmoid(x)

def _layernorm(x, axis=-1, eps=1e-05):
    m = jnp.mean(x, axis=axis, keepdims=True)
    v = jnp.var(x, axis=axis, keepdims=True)
    return (x - m) / jnp.sqrt(v + eps)

def _scatter_add(tgt, idx, src, axis=0):
    return tgt.at[idx].add(src)

def _segment_sum(src, seg, n):
    return jax.ops.segment_sum(src, seg, n)

class _Rng:

    def __init__(self, key):
        self._k = key

    def _next(self):
        self._k, sub = jax.random.split(self._k)
        return sub

    def normal(self, shape):
        return jax.random.normal(self._next(), shape, dtype=jnp.bfloat16)

    def randint(self, lo, hi, shape):
        return jax.random.randint(self._next(), shape, lo, hi, dtype=jnp.int32)

    def uniform(self, shape, lo=0.0, hi=1.0):
        return jax.random.uniform(self._next(), shape, jnp.bfloat16, lo, hi)

    def permutation(self, n):
        return jax.random.permutation(self._next(), n)
kernel_name = 'sequential_preLN__linear_attn_block__mixer_gmlp__prompt'

def setup_inputs():
    _rng = _Rng(jax.random.key(int.from_bytes(__import__("os").urandom(4), "little")))
    _w = lambda a: (lambda t: t.astype(jnp.bfloat16) if jnp.issubdtype(t.dtype, jnp.floating) else t)(jnp.asarray(a))

    def _A_setup():
        B, S, D = (1, 2048, 512)
        return {'x': _w((lambda *s: _rng.normal(s) * 0.05)(B, S, D)), 'wqkv': _w((lambda *s: _rng.normal(s) * 0.05)(D, 3 * D)), 'wo': _w((lambda *s: _rng.normal(s) * 0.05)(D, D))}
    _A_in = _A_setup()

    def _B_setup():
        B, S, D, F = (1, 2048, 512, 1792)
        Fh = F // 2
        return {'x': _w((lambda *s: _rng.normal(s) * 0.05)(B, S, D)), 'w_in': _w((lambda *s: _rng.normal(s) * 0.4)(D, 2 * Fh)), 'w_sp': _w(0.01 * (lambda *s: _rng.normal(s) * 0.4)(S, S)), 'b_sp': _w(1.0 + 0.01 * (lambda *s: _rng.normal(s) * 0.05)(S)), 'w_out': _w((lambda *s: _rng.normal(s) * 0.05)(Fh, D))}
    _B_in = _B_setup()
    return {'A_x': _A_in['x'], 'A_wqkv': _A_in['wqkv'], 'A_wo': _A_in['wo'], 'B_x': _B_in['x'], 'B_w_in': _B_in['w_in'], 'B_w_sp': _B_in['w_sp'], 'B_b_sp': _B_in['b_sp'], 'B_w_out': _B_in['w_out']}

def reference(A_x, A_wqkv, A_wo, B_x, B_w_in, B_w_sp, B_b_sp, B_w_out):

    def _A_ref(x, wqkv, wo):
        B, S, D = x.shape
        H = 32
        Dh = D // H
        qkv = (lambda x, *d: x.transpose(*d))((x @ wqkv).reshape(B, S, 3, H, Dh), 2, 0, 3, 1, 4)
        q, k, v = (qkv[0], qkv[1], qkv[2])
        phi = lambda t: jnp.where(t > 0, t + 1, jnp.exp(t)) + 1e-06
        pq, pk = (phi(q), phi(k))
        kv = jnp.einsum('bhsd,bhse->bhde', pk, v)
        z = jnp.einsum('bhsd->bhd', pk)
        num = jnp.einsum('bhqd,bhde->bhqe', pq, kv)
        den = jnp.einsum('bhqd,bhd->bhq', pq, z)[..., None] + 1e-06
        o = num / den
        return (lambda x, *d: x.transpose(*d))(o, 0, 2, 1, 3).reshape(B, S, D) @ wo

    def _B_ref(x, w_in, w_sp, b_sp, w_out):
        B, S, D = x.shape
        F = w_in.shape[-1]
        Fh = F // 2
        z = _gelu(jnp.einsum('bsd,df->bsf', x, w_in))
        z1 = z[..., :Fh].copy()
        z2 = _layernorm(z[..., Fh:], axis=-1)
        g = jnp.einsum('ts,bsf->btf', w_sp, z2) + b_sp[None, :, None]
        return jnp.einsum('bsf,fd->bsd', z1 * g, w_out)
    x = A_x
    h = x + _A_ref(_layernorm(x, axis=-1), A_wqkv, A_wo)
    h2 = h + _B_ref(_layernorm(h, axis=-1), B_w_in, B_w_sp, B_b_sp, B_w_out)
    return h2
```

```python
import functools

import jax
import jax.numpy as jnp
from jax import lax
import jax.experimental.pallas as pl
import jax.experimental.pallas.tpu as pltpu

_H = 32
_TM = 256
_LANE = 128


def _ln(x):
    m = jnp.mean(x, axis=-1, keepdims=True)
    xc = x - m
    v = jnp.mean(xc * xc, axis=-1, keepdims=True)
    return xc * lax.rsqrt(v + 1e-05)


def _phi(t):
    return jnp.where(t > 0, t + 1.0, jnp.exp(t)) + 1e-06


def _dot(a, b):
    return jnp.dot(a, b, preferred_element_type=jnp.float32)


def _kernel(x_ref, wqkv_ref, wo_ref, win_ref, wsp_ref, bsp_ref, wout_ref, o_ref,
            pq_s, h_s, z1_s, z2_s, kv_s, zs_s, m_s, zbd_s, *, D, FH, DH, TM):
    f32, bf16 = jnp.float32, jnp.bfloat16
    p = pl.program_id(0)
    t = pl.program_id(1)
    rows = pl.ds(pl.multiple_of(t * TM, TM), TM)
    NB = D // _LANE

    @pl.when(p == 0)
    def _phase1():
        @pl.when(t == 0)
        def _():
            kv_s[...] = jnp.zeros(kv_s.shape, f32)
            zs_s[...] = jnp.zeros(zs_s.shape, f32)

        xn = _ln(x_ref[...].astype(f32)).astype(bf16)
        qkv = _dot(xn, wqkv_ref[...])
        pq_s[rows, :] = _phi(qkv[:, :D]).astype(bf16)
        pk = _phi(qkv[:, D:2 * D]).astype(bf16)
        v = qkv[:, 2 * D:].astype(bf16)
        zs_s[...] += jnp.sum(pk.astype(f32), axis=0, keepdims=True)
        for j in range(NB):
            sl = slice(j * _LANE, (j + 1) * _LANE)
            kv_s[j] += lax.dot_general(pk[:, sl], v[:, sl], (((0,), (0,)), ((), ())),
                                       preferred_element_type=f32)

    @pl.when(p == 1)
    def _phase2():
        @pl.when(t == 0)
        def _():
            r = lax.broadcasted_iota(jnp.int32, (_LANE, _LANE), 0) // DH
            c = lax.broadcasted_iota(jnp.int32, (_LANE, _LANE), 1) // DH
            same = r == c
            for j in range(NB):
                sl = slice(j * _LANE, (j + 1) * _LANE)
                kvj = jnp.where(same, kv_s[j], 0.0).astype(bf16)
                m_s[sl, :] = _dot(kvj, wo_ref[sl, :]).astype(bf16)
                zcol = jnp.broadcast_to(zs_s[:, sl], (_LANE, _LANE)).T
                zbd_s[j] = jnp.where(same, zcol, 0.0).astype(bf16)

        pq = pq_s[rows, :]
        den = jnp.concatenate(
            [_dot(pq[:, j * _LANE:(j + 1) * _LANE], zbd_s[j]) for j in range(NB)], axis=1) + 1e-06
        r = (pq.astype(f32) / den).astype(bf16)
        h = x_ref[...].astype(f32) + _dot(r, m_s[...])
        h_s[rows, :] = h
        hn = _ln(h).astype(bf16)
        zz = jax.nn.gelu(_dot(hn, win_ref[...]), approximate=True)
        z1_s[rows, :] = zz[:, :FH].astype(bf16)
        z2_s[rows, :] = _ln(zz[:, FH:]).astype(bf16)

    @pl.when(p == 2)
    def _phase3():
        g = _dot(wsp_ref[...], z2_s[...]) + bsp_ref[...].astype(f32)
        u = (z1_s[rows, :].astype(f32) * g).astype(bf16)
        o_ref[...] = (h_s[rows, :] + _dot(u, wout_ref[...])).astype(o_ref.dtype)


@jax.jit
def pallas_sequential_preLN__linear_attn_block__mixer_gmlp__prompt_kernel(
    A_x: jax.Array,
    A_wqkv: jax.Array,
    A_wo: jax.Array,
    B_x: jax.Array,
    B_w_in: jax.Array,
    B_w_sp: jax.Array,
    B_b_sp: jax.Array,
    B_w_out: jax.Array,
):
    B, S, D = A_x.shape
    assert B == 1
    F = B_w_in.shape[-1]
    FH = F // 2
    DH = D // _H
    TM = _TM
    NT = S // TM
    NB = D // _LANE
    f32, bf16 = jnp.float32, jnp.bfloat16

    x2 = A_x.reshape(S, D)
    bsp = B_b_sp.reshape(S, 1)

    const = lambda p, t: (0, 0)
    out = pl.pallas_call(
        functools.partial(_kernel, D=D, FH=FH, DH=DH, TM=TM),
        grid=(3, NT),
        in_specs=[
            pl.BlockSpec((TM, D), lambda p, t: (jnp.where(p < 2, t, NT - 1), 0)),
            pl.BlockSpec((D, 3 * D), const),
            pl.BlockSpec((D, D), const),
            pl.BlockSpec((D, F), const),
            pl.BlockSpec((TM, S), lambda p, t: (jnp.where(p == 2, t, 0), 0)),
            pl.BlockSpec((TM, 1), lambda p, t: (jnp.where(p == 2, t, 0), 0)),
            pl.BlockSpec((FH, D), const),
        ],
        out_specs=pl.BlockSpec((TM, D), lambda p, t: (jnp.where(p == 2, t, 0), 0)),
        out_shape=jax.ShapeDtypeStruct((S, D), A_x.dtype),
        scratch_shapes=[
            pltpu.VMEM((S, D), bf16),
            pltpu.VMEM((S, D), f32),
            pltpu.VMEM((S, FH), bf16),
            pltpu.VMEM((S, FH), bf16),
            pltpu.VMEM((NB, _LANE, _LANE), f32),
            pltpu.VMEM((1, D), f32),
            pltpu.VMEM((D, D), bf16),
            pltpu.VMEM((NB, _LANE, _LANE), bf16),
        ],
        compiler_params=pltpu.CompilerParams(
            dimension_semantics=("arbitrary", "arbitrary"),
            vmem_limit_bytes=100 * 1024 * 1024,
        ),
    )(x2, A_wqkv, A_wo, B_w_in, B_w_sp, bsp, B_w_out)
    return out.reshape(B, S, D)
```

```python
import functools
import math

import jax
import jax.numpy as jnp
from jax import lax
import jax.experimental.pallas as pl
import jax.experimental.pallas.tpu as pltpu

_H = 32
_TM = 256
_TM3 = 1024
_TO = 256
_LANE = 128


def _ln(x):
    m = jnp.mean(x, axis=-1, keepdims=True)
    xc = x - m
    v = jnp.mean(xc * xc, axis=-1, keepdims=True)
    return xc * lax.rsqrt(v + 1e-05)


def _phi(t):
    return jnp.where(t > 0, t + 1.0, jnp.exp(t)) + 1e-06


def _gelu(x):
    c1 = math.sqrt(2.0 / math.pi)
    u = x * (c1 + (c1 * 0.044715) * (x * x))
    hx = 0.5 * x
    return hx + hx * jnp.tanh(u)


def _dot(a, b):
    return jnp.dot(a, b, preferred_element_type=jnp.float32)


def _kernel(x_hbm, wqkv_hbm, wo_hbm, win_hbm, wsp_hbm, bsp_hbm, wout_hbm, o_hbm,
            x_v, wqkv_v, wo_v, win_v, wsp_v, bsp_v, wout_v, o_v,
            xn_s, pq_s, h_s, hne_s, hno_s, z1_s, z2_s, kv_s, zs_s, m_s, zbd_s,
            sem_x, sem_w, sem_o, *, S, D, FH, DH, TM, TM3, TO):
    f32, bf16 = jnp.float32, jnp.bfloat16
    NB = D // _LANE
    NT = S // TM
    NT3 = S // TM3
    NSUB = TM3 // TO

    def rows_of(t, tm=TM):
        return pl.ds(pl.multiple_of(t * tm, tm), tm)

    def x_copy(t):
        return pltpu.make_async_copy(x_hbm.at[pl.ds(t * TM, TM)], x_v.at[pl.ds(t * TM, TM)], sem_x.at[t])

    def o_copy(t):
        return pltpu.make_async_copy(o_v.at[pl.ds(t * TO, TO)], o_hbm.at[pl.ds(t * TO, TO)], sem_o.at[t])

    def wqkv_copy(j):
        return pltpu.make_async_copy(wqkv_hbm.at[:, pl.ds(j * D, D)], wqkv_v.at[:, pl.ds(j * D, D)], sem_w.at[j])

    c_wo = pltpu.make_async_copy(wo_hbm, wo_v, sem_w.at[3])
    c_win = pltpu.make_async_copy(win_hbm, win_v, sem_w.at[4])
    c_wout = pltpu.make_async_copy(wout_hbm, wout_v, sem_w.at[5])
    c_bsp = pltpu.make_async_copy(bsp_hbm, bsp_v, sem_w.at[6])
    c_wsp = pltpu.make_async_copy(wsp_hbm, wsp_v, sem_w.at[7])

    x_copy(0).start()
    wqkv_copy(1).start(priority=1)
    wqkv_copy(2).start(priority=1)
    wqkv_copy(0).start(priority=1)
    x_copy(1).start(priority=1)
    kv_s[...] = jnp.zeros(kv_s.shape, f32)
    zs_s[...] = jnp.zeros(zs_s.shape, f32)

    def ln_x(t):
        return _ln(x_v[rows_of(t), :].astype(f32)).astype(bf16)

    def qkv_stage(t, xn, nxt, first=False, last=False):
        rows = rows_of(t)
        xn_next = None
        if first:
            wqkv_copy(1).wait()
        k = _dot(xn, wqkv_v[:, D:2 * D])
        if nxt and not first:
            xn_next = ln_x(t + 1)
        pk = _phi(k).astype(bf16)
        if first:
            wqkv_copy(2).wait()
        v = _dot(xn, wqkv_v[:, 2 * D:]).astype(bf16)
        zs_s[...] += jnp.sum(pk.astype(f32), axis=0, keepdims=True)
        if first:
            wqkv_copy(0).wait()
            x_copy(t + 1).wait()
            for tt in range(2, NT):
                x_copy(tt).start()
        if not last:
            q = _dot(xn, wqkv_v[:, :D])
        if first:
            xn_next = ln_x(t + 1)
        for j in range(NB):
            sl = slice(j * _LANE, (j + 1) * _LANE)
            kv_s[j] += lax.dot_general(pk[:, sl], v[:, sl], (((0,), (0,)), ((), ())),
                                       preferred_element_type=f32)
        if last:
            q = _dot(xn, wqkv_v[:, :D])
        pq_s[rows, :] = _phi(q).astype(bf16)
        return xn_next

    x_copy(0).wait()
    xn_s[...] = qkv_stage(0, ln_x(0), True, first=True)
    c_wo.start(priority=1)
    c_win.start(priority=1)

    def phase1(i, carry):
        t = 2 * i + 1
        x_copy(t + 1).wait()
        x_copy(t + 2).wait()
        xn1 = qkv_stage(t, xn_s[...], True)
        xn_s[...] = qkv_stage(t + 1, xn1, True)
        return carry

    lax.fori_loop(0, (NT - 2) // 2, phase1, 0)
    c_wo.wait()
    c_win.wait()
    c_wsp.start(priority=1)
    c_wout.start(priority=1)
    c_bsp.start(priority=1)
    qkv_stage(NT - 1, xn_s[...], False, last=True)

    def den_mm(t):
        pq = pq_s[rows_of(t), :]
        den = jnp.concatenate(
            [_dot(pq[:, j * _LANE:(j + 1) * _LANE], zbd_s[j]) for j in range(NB)], axis=1) + 1e-06
        inv = pl.reciprocal(den, approx=True)
        inv = inv * (2.0 - den * inv)
        return (pq.astype(f32) * inv).astype(bf16)

    def attn_mm(t, r):
        rows = rows_of(t)
        h = x_v[rows, :].astype(f32) + _dot(r, m_s[...])
        h_s[rows, :] = h
        return _ln(h).astype(bf16)

    def z2_mm(t, hn):
        rows = rows_of(t)
        z2 = _gelu(_dot(hn, win_v[:, FH:]))
        z2_s[rows, :] = _ln(z2).astype(bf16)

    def z1_mm(t, hn):
        rows = rows_of(t)
        z1_s[rows, :] = _dot(hn, win_v[:, :FH]).astype(bf16)

    r = lax.broadcasted_iota(jnp.int32, (_LANE, _LANE), 0) // DH
    c = lax.broadcasted_iota(jnp.int32, (_LANE, _LANE), 1) // DH
    same = r == c
    for j in range(NB):
        sl = slice(j * _LANE, (j + 1) * _LANE)
        zcol = jnp.broadcast_to(zs_s[:, sl], (_LANE, _LANE)).T
        zbd_s[j] = jnp.where(same, zcol, 0.0).astype(bf16)
    r0 = den_mm(0)
    for j in range(NB):
        sl = slice(j * _LANE, (j + 1) * _LANE)
        kvj = jnp.where(same, kv_s[j], 0.0).astype(bf16)
        m_s[sl, :] = _dot(kvj, wo_v[sl, :]).astype(bf16)
    r1 = den_mm(1)
    hne_s[rows_of(0), :] = attn_mm(0, r0)
    hno_s[rows_of(0), :] = attn_mm(1, r1)

    def phase2(i, carry):
        t = 2 * i
        hn0 = hne_s[rows_of(i), :]
        ra = den_mm(t + 2)
        z2_mm(t, hn0)
        hne_s[rows_of(i + 1), :] = attn_mm(t + 2, ra)
        z1_mm(t, hn0)
        hn1 = hno_s[rows_of(i), :]
        rb = den_mm(t + 3)
        z2_mm(t + 1, hn1)
        hno_s[rows_of(i + 1), :] = attn_mm(t + 3, rb)
        z1_mm(t + 1, hn1)
        return carry

    lax.fori_loop(0, (NT - 2) // 2, phase2, 0)
    for t, ref in ((NT - 2, hne_s), (NT - 1, hno_s)):
        hn = ref[rows_of(NT // 2 - 1), :]
        z2_mm(t, hn)
        z1_mm(t, hn)

    c_wout.wait()
    c_bsp.wait()
    c_wsp.wait()

    def phase3(t, carry):
        rows = rows_of(t, TM3)
        b = bsp_v[rows].astype(f32).reshape(1, TM3)
        bcol = jnp.broadcast_to(b, (_LANE, TM3)).T
        bfull = jnp.concatenate([bcol] * (FH // _LANE), axis=1)
        g = _dot(wsp_v[rows, :], z2_s[...]) + bfull
        u = (_gelu(z1_s[rows, :].astype(f32)) * g).astype(bf16)
        for i in range(NSUB):
            sub = rows_of(t * NSUB + i, TO)
            o_v[sub, :] = (h_s[sub, :] + _dot(u[i * TO:(i + 1) * TO], wout_v[...])).astype(o_v.dtype)
            o_copy(t * NSUB + i).start()
        return carry

    lax.fori_loop(0, NT3, phase3, 0)
    for t in range(S // TO):
        o_copy(t).wait()


@jax.jit
def pallas_sequential_preLN__linear_attn_block__mixer_gmlp__prompt_kernel(
    A_x: jax.Array,
    A_wqkv: jax.Array,
    A_wo: jax.Array,
    B_x: jax.Array,
    B_w_in: jax.Array,
    B_w_sp: jax.Array,
    B_b_sp: jax.Array,
    B_w_out: jax.Array,
):
    B, S, D = A_x.shape
    assert B == 1
    F = B_w_in.shape[-1]
    FH = F // 2
    DH = D // _H
    TM = _TM
    TM3 = _TM3
    TO = _TO
    NT = S // TM
    NB = D // _LANE
    f32, bf16 = jnp.float32, jnp.bfloat16

    x2 = A_x.reshape(S, D)

    anyspec = pl.BlockSpec(memory_space=pl.ANY)
    out = pl.pallas_call(
        functools.partial(_kernel, S=S, D=D, FH=FH, DH=DH, TM=TM, TM3=TM3, TO=TO),
        in_specs=[anyspec] * 7,
        out_specs=anyspec,
        out_shape=jax.ShapeDtypeStruct((S, D), A_x.dtype),
        scratch_shapes=[
            pltpu.VMEM((S, D), bf16),
            pltpu.VMEM((D, 3 * D), bf16),
            pltpu.VMEM((D, D), bf16),
            pltpu.VMEM((D, F), bf16),
            pltpu.VMEM((S, S), bf16),
            pltpu.VMEM((S,), bf16),
            pltpu.VMEM((FH, D), bf16),
            pltpu.VMEM((S, D), bf16),
            pltpu.VMEM((TM, D), bf16),
            pltpu.VMEM((S, D), bf16),
            pltpu.VMEM((S, D), f32),
            pltpu.VMEM((S // 2, D), bf16),
            pltpu.VMEM((S // 2, D), bf16),
            pltpu.VMEM((S, FH), bf16),
            pltpu.VMEM((S, FH), bf16),
            pltpu.VMEM((NB, _LANE, _LANE), f32),
            pltpu.VMEM((1, D), f32),
            pltpu.VMEM((D, D), bf16),
            pltpu.VMEM((NB, _LANE, _LANE), bf16),
            pltpu.SemaphoreType.DMA((NT,)),
            pltpu.SemaphoreType.DMA((8,)),
            pltpu.SemaphoreType.DMA((S // TO,)),
        ],
        compiler_params=pltpu.CompilerParams(
            vmem_limit_bytes=100 * 1024 * 1024,
        ),
    )(x2, A_wqkv, A_wo, B_w_in, B_w_sp, B_b_sp, B_w_out)
    return out.reshape(B, S, D)
```

```python
import functools
import math

import jax
import jax.numpy as jnp
from jax import lax
import jax.experimental.pallas as pl
import jax.experimental.pallas.tpu as pltpu

_H = 32
_TM = 256
_TM3 = 1024
_TO = 256
_LANE = 128


def _ln(x):
    m = jnp.mean(x, axis=-1, keepdims=True)
    xc = x - m
    v = jnp.mean(xc * xc, axis=-1, keepdims=True)
    return xc * lax.rsqrt(v + 1e-05)


def _phi(t):
    return jnp.where(t > 0, t + 1.0, jnp.exp(t)) + 1e-06


def _gelu(x):
    c1 = math.sqrt(2.0 / math.pi)
    u = x * (c1 + (c1 * 0.044715) * (x * x))
    hx = 0.5 * x
    return hx + hx * jnp.tanh(u)


def _dot(a, b):
    return jnp.dot(a, b, preferred_element_type=jnp.float32)


def _kernel(x_hbm, wqkv_hbm, wo_hbm, win_hbm, wsp_hbm, bsp_hbm, wout_hbm, o_hbm,
            x_v, wqkv_v, wo_v, win_v, wsp_v, bsp_v, wout_v, o_v,
            xn_s, pq_s, h_s, hne_s, hno_s, z1_s, z2_s, kv_s, zs_s, m_s, zbd_s,
            sem_x, sem_w, sem_o, *, S, D, FH, DH, TM, TM3, TO):
    f32, bf16 = jnp.float32, jnp.bfloat16
    NB = D // _LANE
    NT = S // TM
    NT3 = S // TM3
    NSUB = TM3 // TO

    def rows_of(t, tm=TM):
        return pl.ds(pl.multiple_of(t * tm, tm), tm)

    def x_copy(t):
        return pltpu.make_async_copy(x_hbm.at[pl.ds(t * TM, TM)], x_v.at[pl.ds(t * TM, TM)],
                                     sem_x.at[t])

    def o_copy(t):
        return pltpu.make_async_copy(o_v.at[pl.ds(t * TO, TO)], o_hbm.at[pl.ds(t * TO, TO)],
                                     sem_o.at[t])

    def wqkv_copy(j):
        return pltpu.make_async_copy(wqkv_hbm.at[:, pl.ds(j * D, D)],
                                     wqkv_v.at[:, pl.ds(j * D, D)], sem_w.at[j])

    c_wo = pltpu.make_async_copy(wo_hbm, wo_v, sem_w.at[3])
    c_win = pltpu.make_async_copy(win_hbm, win_v, sem_w.at[4])
    c_wout = pltpu.make_async_copy(wout_hbm, wout_v, sem_w.at[5])
    c_bsp = pltpu.make_async_copy(bsp_hbm, bsp_v, sem_w.at[6])
    c_wsp = pltpu.make_async_copy(wsp_hbm, wsp_v, sem_w.at[7])

    x_copy(0).start()
    wqkv_copy(1).start(priority=1)
    wqkv_copy(2).start(priority=1)
    wqkv_copy(0).start(priority=1)
    x_copy(1).start(priority=1)
    kv_s[...] = jnp.zeros(kv_s.shape, f32)
    zs_s[...] = jnp.zeros(zs_s.shape, f32)

    def ln_x(t):
        return _ln(x_v[rows_of(t), :].astype(f32)).astype(bf16)

    def qkv_stage(t, xn, nxt, first=False, last=False):
        rows = rows_of(t)
        xn_next = None
        if first:
            wqkv_copy(1).wait()
        k = _dot(xn, wqkv_v[:, D:2 * D])
        if nxt and not first:
            xn_next = ln_x(t + 1)
        pk = _phi(k).astype(bf16)
        if first:
            wqkv_copy(2).wait()
        v = _dot(xn, wqkv_v[:, 2 * D:]).astype(bf16)
        zs_s[...] += jnp.sum(pk.astype(f32), axis=0, keepdims=True)
        if first:
            wqkv_copy(0).wait()
            x_copy(t + 1).wait()
            for tt in range(2, NT):
                x_copy(tt).start()
        if not last:
            q = _dot(xn, wqkv_v[:, :D])
        if first:
            xn_next = ln_x(t + 1)
        for j in range(NB):
            sl = slice(j * _LANE, (j + 1) * _LANE)
            kv_s[j] += lax.dot_general(pk[:, sl], v[:, sl], (((0,), (0,)), ((), ())),
                                       preferred_element_type=f32)
        if last:
            q = _dot(xn, wqkv_v[:, :D])
        pq_s[rows, :] = _phi(q).astype(bf16)
        return xn_next

    x_copy(0).wait()
    xn_s[...] = qkv_stage(0, ln_x(0), True, first=True)
    c_wo.start(priority=1)
    c_win.start(priority=1)

    def phase1(i, carry):
        t = 2 * i + 1
        x_copy(t + 1).wait()
        x_copy(t + 2).wait()
        xn1 = qkv_stage(t, xn_s[...], True)
        xn_s[...] = qkv_stage(t + 1, xn1, True)
        return carry

    lax.fori_loop(0, (NT - 2) // 2, phase1, 0)
    c_wo.wait()
    c_win.wait()
    c_wsp.start(priority=1)
    c_wout.start(priority=1)
    c_bsp.start(priority=1)
    qkv_stage(NT - 1, xn_s[...], False, last=True)

    def den_mm(t):
        pq = pq_s[rows_of(t), :]
        den = jnp.concatenate(
            [_dot(pq[:, j * _LANE:(j + 1) * _LANE], zbd_s[j]) for j in range(NB)], axis=1) + 1e-06
        inv = pl.reciprocal(den, approx=True)
        inv = inv * (2.0 - den * inv)
        return (pq.astype(f32) * inv).astype(bf16)

    def attn_mm(t, r):
        rows = rows_of(t)
        h = x_v[rows, :].astype(f32) + _dot(r, m_s[...])
        h_s[rows, :] = h
        return _ln(h).astype(bf16)

    def z2_mm(t, hn):
        rows = rows_of(t)
        z2 = _gelu(_dot(hn, win_v[:, FH:]))
        z2_s[rows, :] = _ln(z2).astype(bf16)

    def z1_mm(t, hn):
        rows = rows_of(t)
        z1_s[rows, :] = _dot(hn, win_v[:, :FH]).astype(bf16)

    r = lax.broadcasted_iota(jnp.int32, (_LANE, _LANE), 0) // DH
    c = lax.broadcasted_iota(jnp.int32, (_LANE, _LANE), 1) // DH
    same = r == c
    for j in range(NB):
        sl = slice(j * _LANE, (j + 1) * _LANE)
        zcol = jnp.broadcast_to(zs_s[:, sl], (_LANE, _LANE)).T
        zbd_s[j] = jnp.where(same, zcol, 0.0).astype(bf16)
    r0 = den_mm(0)
    for j in range(NB):
        sl = slice(j * _LANE, (j + 1) * _LANE)
        kvj = jnp.where(same, kv_s[j], 0.0).astype(bf16)
        m_s[sl, :] = _dot(kvj, wo_v[sl, :]).astype(bf16)
    r1 = den_mm(1)
    hne_s[rows_of(0), :] = attn_mm(0, r0)
    hno_s[rows_of(0), :] = attn_mm(1, r1)

    def phase2(i, carry):
        t = 2 * i
        hn0 = hne_s[rows_of(i), :]
        ra = den_mm(t + 2)
        z2_mm(t, hn0)
        hne_s[rows_of(i + 1), :] = attn_mm(t + 2, ra)
        z1_mm(t, hn0)
        hn1 = hno_s[rows_of(i), :]
        rb = den_mm(t + 3)
        z2_mm(t + 1, hn1)
        hno_s[rows_of(i + 1), :] = attn_mm(t + 3, rb)
        z1_mm(t + 1, hn1)
        return carry

    lax.fori_loop(0, (NT - 2) // 2, phase2, 0)
    for t, ref in ((NT - 2, hne_s), (NT - 1, hno_s)):
        hn = ref[rows_of(NT // 2 - 1), :]
        z2_mm(t, hn)
        z1_mm(t, hn)

    c_wout.wait()
    c_bsp.wait()
    c_wsp.wait()

    def phase3(t, carry):
        rows = rows_of(t, TM3)
        b = bsp_v[rows].astype(f32).reshape(1, TM3)
        bcol = jnp.broadcast_to(b, (_LANE, TM3)).T
        bfull = jnp.concatenate([bcol] * (FH // _LANE), axis=1)
        g = _dot(wsp_v[rows, :], z2_s[...]) + bfull
        u = (_gelu(z1_s[rows, :].astype(f32)) * g).astype(bf16)
        for i in range(NSUB):
            sub = rows_of(t * NSUB + i, TO)
            o_v[sub, :] = (h_s[sub, :]
                           + _dot(u[i * TO:(i + 1) * TO], wout_v[...])).astype(o_v.dtype)
            o_copy(t * NSUB + i).start()
        return carry

    lax.fori_loop(0, NT3, phase3, 0)
    for t in range(S // TO):
        o_copy(t).wait()


@jax.jit
def pallas_sequential_preLN__linear_attn_block__mixer_gmlp__prompt_kernel(
    A_x: jax.Array,
    A_wqkv: jax.Array,
    A_wo: jax.Array,
    B_x: jax.Array,
    B_w_in: jax.Array,
    B_w_sp: jax.Array,
    B_b_sp: jax.Array,
    B_w_out: jax.Array,
):
    del B_x
    B, S, D = A_x.shape
    F = B_w_in.shape[-1]
    FH = F // 2
    DH = D // _H
    TM, TM3, TO = _TM, _TM3, _TO
    NT = S // TM
    NB = D // _LANE
    assert B == 1 and S % TM3 == 0 and TM3 % TO == 0 and S % (2 * TM) == 0 and NT >= 4
    assert D % _LANE == 0 and FH % _LANE == 0 and _LANE % DH == 0
    f32, bf16 = jnp.float32, jnp.bfloat16

    anyspec = pl.BlockSpec(memory_space=pl.ANY)
    out = pl.pallas_call(
        functools.partial(_kernel, S=S, D=D, FH=FH, DH=DH, TM=TM, TM3=TM3, TO=TO),
        in_specs=[anyspec] * 7,
        out_specs=anyspec,
        out_shape=jax.ShapeDtypeStruct((S, D), A_x.dtype),
        scratch_shapes=[
            pltpu.VMEM((S, D), bf16),
            pltpu.VMEM((D, 3 * D), bf16),
            pltpu.VMEM((D, D), bf16),
            pltpu.VMEM((D, F), bf16),
            pltpu.VMEM((S, S), bf16),
            pltpu.VMEM((S,), bf16),
            pltpu.VMEM((FH, D), bf16),
            pltpu.VMEM((S, D), bf16),
            pltpu.VMEM((TM, D), bf16),
            pltpu.VMEM((S, D), bf16),
            pltpu.VMEM((S, D), f32),
            pltpu.VMEM((S // 2, D), bf16),
            pltpu.VMEM((S // 2, D), bf16),
            pltpu.VMEM((S, FH), bf16),
            pltpu.VMEM((S, FH), bf16),
            pltpu.VMEM((NB, _LANE, _LANE), f32),
            pltpu.VMEM((1, D), f32),
            pltpu.VMEM((D, D), bf16),
            pltpu.VMEM((NB, _LANE, _LANE), bf16),
            pltpu.SemaphoreType.DMA((NT,)),
            pltpu.SemaphoreType.DMA((8,)),
            pltpu.SemaphoreType.DMA((S // TO,)),
        ],
        compiler_params=pltpu.CompilerParams(
            vmem_limit_bytes=100 * 1024 * 1024,
        ),
    )(A_x.reshape(S, D), A_wqkv, A_wo, B_w_in, B_w_sp, B_b_sp, B_w_out)
    return out.reshape(B, S, D)
```
